```python
import os as _os
_os.environ.setdefault("JAX_PLATFORMS", "cpu")
import jax
import jax.numpy as jnp

def _softmax(x, axis=-1):
    return jax.nn.softmax(x, axis=axis)
def _gelu(x):
    return jax.nn.gelu(x, approximate=True)
def _silu(x):
    return jax.nn.silu(x)
def _sigmoid(x):
    return jax.nn.sigmoid(x)
def _layernorm(x, axis=-1, eps=1e-5):
    m = jnp.mean(x, axis=axis, keepdims=True)
    v = jnp.var(x, axis=axis, keepdims=True)
    return (x - m) / jnp.sqrt(v + eps)
def _scatter_add(tgt, idx, src, axis=0):
    return tgt.at[idx].add(src)
def _segment_sum(src, seg, n):
    return jax.ops.segment_sum(src, seg, n)
class _Rng:
    def __init__(self, key):
        self._k = key
    def _next(self):
        self._k, sub = jax.random.split(self._k)
        return sub
    def normal(self, shape):
        return jax.random.normal(self._next(), shape, dtype=jnp.bfloat16)
    def randint(self, lo, hi, shape):
        return jax.random.randint(self._next(), shape, lo, hi, dtype=jnp.int32)
    def uniform(self, shape, lo=0.0, hi=1.0):
        return jax.random.uniform(self._next(), shape, jnp.bfloat16, lo, hi)
    def permutation(self, n):
        return jax.random.permutation(self._next(), n)


kernel_name = 'concat_heads__gqa_block_cached__gqa_block_cached__near_ridge'

def setup_inputs():
    _rng = _Rng(jax.random.key(int.from_bytes(__import__("os").urandom(4), "little")))
    _w = (lambda a: (lambda t: t.astype(jnp.bfloat16) if jnp.issubdtype(t.dtype, jnp.floating) else t)(jnp.asarray(a)))
    def _A_setup():
        B, Sq, D = 8, 240, 640
        Hq, Hkv, Sk, Dh = 32, 32, 1024, 192
        assert Hq % Hkv == 0, (Hq, Hkv)
        return {
            "x": _w((lambda *s: _rng.normal(s) * 0.8)(B, Sq, D)),
            "k_cache": _w((lambda *s: _rng.normal(s) * 0.8)(B, Hkv, Sk, Dh)),
            "v_cache": _w((lambda *s: _rng.normal(s) * 0.05)(B, Hkv, Sk, Dh)),
            "wq": _w((lambda *s: _rng.normal(s) * 0.8)(D, Hq * Dh) * (D ** -0.5)),
            "wo": _w((lambda *s: _rng.normal(s) * 0.05)(Hq * Dh, D) * ((Hq * Dh) ** -0.5)),
        }
    _A_in = _A_setup()

    def _B_setup():
        B, Sq, D = 8, 240, 640
        Hq, Hkv, Sk, Dh = 32, 32, 1024, 192
        assert Hq % Hkv == 0, (Hq, Hkv)
        return {
            "x": _w((lambda *s: _rng.normal(s) * 0.8)(B, Sq, D)),
            "k_cache": _w((lambda *s: _rng.normal(s) * 0.8)(B, Hkv, Sk, Dh)),
            "v_cache": _w((lambda *s: _rng.normal(s) * 0.05)(B, Hkv, Sk, Dh)),
            "wq": _w((lambda *s: _rng.normal(s) * 0.8)(D, Hq * Dh) * (D ** -0.5)),
            "wo": _w((lambda *s: _rng.normal(s) * 0.05)(Hq * Dh, D) * ((Hq * Dh) ** -0.5)),
        }
    _B_in = _B_setup()

    return {
        "A_x": _A_in["x"],
        "A_k_cache": _A_in["k_cache"],
        "A_v_cache": _A_in["v_cache"],
        "A_wq": _A_in["wq"],
        "A_wo": _A_in["wo"],
        "B_x": _B_in["x"],
        "B_k_cache": _B_in["k_cache"],
        "B_v_cache": _B_in["v_cache"],
        "B_wq": _B_in["wq"],
        "B_wo": _B_in["wo"],
    }

def reference(A_x, A_k_cache, A_v_cache, A_wq, A_wo, B_x, B_k_cache, B_v_cache, B_wq, B_wo):
    def _A_ref(x, k_cache, v_cache, wq, wo):
        B, Sq, D = x.shape
        Hq, Dh = 32, 192
        Hkv = k_cache.shape[1]
        rep = Hq // Hkv
        q = (lambda x, *d: x.transpose(*d))((x @ wq).reshape(B, Sq, Hq, Dh), 0, 2, 1, 3)
        k = jnp.repeat(k_cache, rep, axis=1)
        v = jnp.repeat(v_cache, rep, axis=1)
        scores = jnp.einsum("bhqd,bhkd->bhqk", q, k) * (Dh ** -0.5)
        p = _softmax(scores, axis=-1)
        o = jnp.einsum("bhqk,bhkd->bhqd", p, v)
        return (lambda x, *d: x.transpose(*d))(o, 0, 2, 1, 3).reshape(B, Sq, Hq * Dh) @ wo

    def _B_ref(x, k_cache, v_cache, wq, wo):
        B, Sq, D = x.shape
        Hq, Dh = 32, 192
        Hkv = k_cache.shape[1]
        rep = Hq // Hkv
        q = (lambda x, *d: x.transpose(*d))((x @ wq).reshape(B, Sq, Hq, Dh), 0, 2, 1, 3)
        k = jnp.repeat(k_cache, rep, axis=1)
        v = jnp.repeat(v_cache, rep, axis=1)
        scores = jnp.einsum("bhqd,bhkd->bhqk", q, k) * (Dh ** -0.5)
        p = _softmax(scores, axis=-1)
        o = jnp.einsum("bhqk,bhkd->bhqd", p, v)
        return (lambda x, *d: x.transpose(*d))(o, 0, 2, 1, 3).reshape(B, Sq, Hq * Dh) @ wo

    a = _A_ref(A_x, A_k_cache, A_v_cache, A_wq, A_wo)
    b = _B_ref(B_x, B_k_cache, B_v_cache, B_wq, B_wo)
    return jnp.concatenate([a, b], axis=-1)
```

```python
import functools

import jax
import jax.numpy as jnp
from jax.experimental import pallas as pl
from jax.experimental.pallas import tpu as pltpu

BF16 = jnp.bfloat16
F32 = jnp.float32
LOG2E = 1.4426950408889634
NN = (((1,), (0,)), ((), ()))
NT = (((1,), (1,)), ((), ()))


def _mm(a, b, dn=NN):
    return jax.lax.dot_general(a, b, dn, preferred_element_type=F32)


def _order_T2(nu):
    seq = []
    for g in range(0, nu, 2):
        a, c = g, g + 1
        seq += [('QP', a), ('QP', c), ('QK', a, 0), ('QK', a, 1), ('SM', a, 0), ('QK', c, 0), ('SM', a, 1),
                ('QK', c, 1), ('SM', c, 0), ('PV', a, 0), ('SM', c, 1), ('PV', a, 1), ('PV', c, 0), ('FIN', a),
                ('PV', c, 1), ('OP', a), ('FIN', c), ('OP', c)]
    return seq


ORD = {'T2': _order_T2}


def make(hps=2, order='T2', order1='T2', start_pos=1, start_pos1=1, vmem=110, flags=None, dbc=True):
    NS = 2 * hps

    def kern(xa, ka, va, wqa, woa, xb, kb, vb, wqb, wob, out_hbm,
             xbuf, kvbuf, wqbuf, wobuf, acc_ref, obuf,
             xsem, kvsem, wqsem, wosem, osem, *, Dh, NP):
        XH = (xa, xb); KVH = ((ka, kb), (va, vb)); WQH = (wqa, wqb); WOH = (woa, wob)
        B, Sq, D = xa.shape
        PW = 2 * Dh
        NG = NP // hps
        scale = float(Dh ** -0.5 * LOG2E)

        def chunk_start(p, b, cs):
            for r in range(2):
                pltpu.make_async_copy(XH[r].at[b], xbuf.at[cs, r], xsem.at[cs]).start()
            for kv in range(2):
                for r in range(2):
                    pltpu.make_async_copy(KVH[kv][r].at[b, pl.ds(pl.multiple_of(p * 2, 2), 2)],
                                          kvbuf.at[cs, kv, r], kvsem.at[cs]).start()

        def chunk_wait(cs):
            pltpu.make_async_copy(xbuf.at[cs], xbuf.at[cs], xsem.at[cs]).wait()
            pltpu.make_async_copy(kvbuf.at[cs], kvbuf.at[cs], kvsem.at[cs]).wait()

        def w_full_start(p, ws):
            c0 = p * PW
            for r in range(2):
                pltpu.make_async_copy(WQH[r].at[:, pl.ds(c0, PW)], wqbuf.at[ws, r], wqsem.at[ws]).start()
            for r in range(2):
                pltpu.make_async_copy(WOH[r].at[pl.ds(c0, PW), :], wobuf.at[ws, r], wosem.at[ws]).start()

        def w_slice_start(p, b, ws):
            rq = D // B; ro = PW // B
            c0 = pl.multiple_of(p * PW, 128)
            q0 = pl.multiple_of(b * rq, rq); o0 = pl.multiple_of(b * ro, ro)
            for r in range(2):
                pltpu.make_async_copy(WQH[r].at[pl.ds(q0, rq), pl.ds(c0, PW)],
                                      wqbuf.at[ws, r, pl.ds(q0, rq)], wqsem.at[ws]).start()
                pltpu.make_async_copy(WOH[r].at[pl.ds(c0 + o0, ro), :],
                                      wobuf.at[ws, r, pl.ds(o0, ro)], wosem.at[ws]).start()

        def w_wait(ws):
            pltpu.make_async_copy(wqbuf.at[ws], wqbuf.at[ws], wqsem.at[ws]).wait()
            pltpu.make_async_copy(wobuf.at[ws], wobuf.at[ws], wosem.at[ws]).wait()

        def o_cp(b, slot):
            return pltpu.make_async_copy(obuf.at[slot], out_hbm.at[b], osem.at[slot])

        def compute(first, b, cs0, ws0, npair, seq, hook):
            st = {}

            def QP(u):
                r, j = u % 2, u // 2
                qp = _mm(xbuf[cs0 + j, r], wqbuf[ws0 + j, r]) * scale
                st['q', u] = qp.astype(BF16)

            def QK(u, h):
                r, j = u % 2, u // 2
                q = st['q', u][:, h * Dh:(h + 1) * Dh]
                st['s', u, h] = _mm(q, kvbuf[cs0 + j, 0, r, h])

            def SM(u, h):
                s = st['s', u, h]
                m = jnp.max(s, axis=-1, keepdims=True)
                e = jnp.exp2(s - m)
                st['l', u, h] = jnp.sum(e, axis=-1, keepdims=True)
                st['p', u, h] = e.astype(BF16)

            def PV(u, h):
                r, j = u % 2, u // 2
                st['o', u, h] = _mm(kvbuf[cs0 + j, 1, r, h], st['p', u, h], NT)

            def FIN(u):
                ot = jnp.concatenate([st['o', u, 0], st['o', u, 1]], axis=0)
                il0 = 1.0 / st['l', u, 0]; il1 = 1.0 / st['l', u, 1]
                lane = jax.lax.broadcasted_iota(jnp.int32, (Sq, 2 * Dh), 1)
                il = jnp.where(lane < Dh, il0, il1)
                st['on', u] = (ot.T * il).astype(BF16)

            def OP(u):
                r, j = u % 2, u // 2
                y = _mm(st['on', u], wobuf[ws0 + j, r])
                if j < npair - 1:
                    st['y', r] = y if j == 0 else st['y', r] + y
                else:
                    if j > 0:
                        y = st['y', r] + y
                    old = acc_ref[b, :, r * D:(r + 1) * D]
                    if first is not False:
                        old = jnp.where(first, 0.0, old)
                    acc_ref[b, :, r * D:(r + 1) * D] = y + old

            F = dict(QP=QP, QK=QK, SM=SM, PV=PV, FIN=FIN, OP=OP)
            for i, (f, *a) in enumerate(seq):
                hook(i)
                F[f](*a)

        chunk_start(0, 0, 0)
        w_full_start(0, 0)

        def p1_outer(p, c):
            w_wait(p)

            @pl.when(p == 0)
            def _():
                for k in range(1, hps):
                    chunk_start(k // B, k % B, k)

            def inner(b, c):
                cidx = p * B + b
                cs = jax.lax.rem(cidx, NS)
                wrap = (b + hps >= B)
                np_ = jnp.where(wrap, p + 1, p); nb = jnp.where(wrap, b + hps - B, b + hps)
                is_tr = jnp.logical_and(wrap, p == hps - 1)
                np_ = jnp.where(is_tr, hps + (b + hps - B), np_); nb = jnp.where(is_tr, 0, nb)

                def hook(i):
                    if i == start_pos1:
                        chunk_start(np_, nb, jax.lax.rem(cidx + hps, NS))
                        pa = 2 * p + 1
                        w_slice_start(pa, b, pa)

                        @pl.when(pa + 1 < 2 * hps)
                        def _():
                            w_slice_start(pa + 1, b, pa + 1)

                chunk_wait(cs)
                compute(p == 0, b, cs, p, 1, ORD[order1](2), hook)
                return c

            jax.lax.fori_loop(0, B, inner, 0)
            return c

        jax.lax.fori_loop(0, hps, p1_outer, 0)

        def finalize(g, b):
            @pl.when(g == NG - 1)
            def _():
                so = jax.lax.rem(b, 2)

                @pl.when(b >= 2)
                def _():
                    o_cp(b - 2, so).wait()

                RC = 48

                def cvt(i, c):
                    rows = pl.ds(pl.multiple_of(i * RC, RC), RC)
                    obuf[so, rows, :] = acc_ref[b, rows, :].astype(BF16)
                    return c

                jax.lax.fori_loop(0, Sq // RC, cvt, 0)
                o_cp(b, so).start()

        def p2_outer(g, c):
            gs = jax.lax.rem(g, 2)
            ws0 = gs * hps
            for j in range(hps):
                w_wait(ws0 + j)

            def inner(b, c):
                ks = jax.lax.rem(b, 2)
                cs0 = ks * hps
                last_b = (b == B - 1)
                nb = jnp.where(last_b, 0, b + 1)
                ng = jnp.minimum(jnp.where(last_b, g + 1, g), NG - 1)
                g1 = jnp.minimum(g + 1, NG - 1)

                def hook(i):
                    if i == start_pos:
                        for j in range(hps):
                            chunk_start(ng * hps + j, nb, (1 - ks) * hps + j)
                        for j in range(hps):
                            w_slice_start(g1 * hps + j, b, (1 - gs) * hps + j)

                for j in range(hps):
                    chunk_wait(cs0 + j)
                compute(False, b, cs0, ws0, hps, ORD[order](2 * hps), hook)
                finalize(g, b)
                return c

            jax.lax.fori_loop(0, B, inner, 0)
            return c

        jax.lax.fori_loop(1, NG, p2_outer, 0)
        for j in range(hps):
            chunk_wait(j)
        for j in range(hps):
            w_wait((NG % 2) * hps + j)
        o_cp(B - 2, (B - 2) % 2).wait()
        o_cp(B - 1, (B - 1) % 2).wait()

    def fn(A_x, A_k, A_v, A_wq, A_wo, B_x, B_k, B_v, B_wq, B_wo):
        B, Sq, D = A_x.shape
        _, H, Sk, Dh = A_k.shape
        NP = H // 2
        assert H % (2 * hps) == 0 and NP // hps >= 2 and B % 2 == 0 and B >= hps
        kt = lambda a: jnp.swapaxes(a, 2, 3)
        anys = pl.BlockSpec(memory_space=pl.ANY)
        return pl.pallas_call(
            functools.partial(kern, Dh=Dh, NP=NP),
            in_specs=[anys] * 10,
            out_specs=anys,
            out_shape=jax.ShapeDtypeStruct((B, Sq, 2 * D), A_x.dtype),
            scratch_shapes=[
                pltpu.VMEM((NS, 2, Sq, D), BF16),
                pltpu.VMEM((NS, 2, 2, 2, Dh, Sk), BF16),
                pltpu.VMEM((NS, 2, D, 2 * Dh), BF16),
                pltpu.VMEM((NS, 2, 2 * Dh, D), BF16),
                pltpu.VMEM((B, Sq, 2 * D), F32),
                pltpu.VMEM((2, Sq, 2 * D), BF16),
                pltpu.SemaphoreType.DMA((NS,)),
                pltpu.SemaphoreType.DMA((NS,)),
                pltpu.SemaphoreType.DMA((NS,)),
                pltpu.SemaphoreType.DMA((NS,)),
                pltpu.SemaphoreType.DMA((2,)),
            ],
            compiler_params=pltpu.CompilerParams(vmem_limit_bytes=vmem * 1024 * 1024, flags=flags,
                                                 disable_bounds_checks=dbc),
        )(A_x, kt(A_k), kt(A_v), A_wq, A_wo, B_x, kt(B_k), kt(B_v), B_wq, B_wo)

    return fn


_impl = make(2)


@jax.jit
def pallas_concat_heads__gqa_block_cached__gqa_block_cached__near_ridge_kernel(
        A_x, A_k_cache, A_v_cache, A_wq, A_wo, B_x, B_k_cache, B_v_cache, B_wq, B_wo):
    return _impl(A_x, A_k_cache, A_v_cache, A_wq, A_wo, B_x, B_k_cache, B_v_cache, B_wq, B_wo)
```

```python
import functools

import jax
import jax.numpy as jnp
from jax.experimental import pallas as pl
from jax.experimental.pallas import tpu as pltpu

BF16 = jnp.bfloat16
F32 = jnp.float32
LOG2E = 1.4426950408889634
NN = (((1,), (0,)), ((), ()))
NT = (((1,), (1,)), ((), ()))

HPS = 2
NFG = 2
QS = 128

_ORDER_MAIN = (
    ('QP', 0), ('QP', 1), ('DX',), ('QK', 0, 0), ('QK', 0, 1), ('SM', 0, 1), ('SM', 0, 0), ('PVT', 0, 0),
    ('QK', 1, 0), ('SM', 1, 0), ('PVT', 0, 1), ('DK',), ('DV',), ('PVN', 0, 0), ('PVA', 0, 0), ('DW',),
    ('QK', 1, 1), ('PVA', 0, 1), ('PVN', 0, 1), ('PVA', 1, 0), ('PVN', 1, 0), ('PVT', 1, 0), ('FIN', 0),
    ('OP', 0), ('SM', 1, 1), ('PVA', 1, 1), ('PVN', 1, 1), ('PVT', 1, 1), ('QP', 2), ('FIN', 1),
    ('QK', 2, 0), ('OP', 1), ('QK', 2, 1), ('QP', 3), ('QK', 3, 0), ('SM', 2, 1), ('QK', 3, 1),
    ('SM', 2, 0), ('PVA', 2, 0), ('PVN', 2, 0), ('PVN', 2, 1), ('SM', 3, 1), ('SM', 3, 0), ('PVT', 2, 0),
    ('PVA', 2, 1), ('PVT', 2, 1), ('PVN', 3, 0), ('PVT', 3, 0), ('FIN', 2), ('PVA', 3, 0), ('PVA', 3, 1),
    ('PVN', 3, 1), ('PVT', 3, 1), ('OP', 2), ('FIN', 3), ('OP', 3),
)
_ORDER_RAMP = (
    ('QP', 0), ('QK', 0, 0), ('SM', 0, 0), ('DK',), ('QK', 0, 1), ('QP', 1), ('QK', 1, 0), ('DV',),
    ('SM', 0, 1), ('DX',), ('PVA', 0, 0), ('SM', 1, 0), ('PVN', 0, 0), ('QK', 1, 1), ('DW',),
    ('PVT', 0, 0), ('PVA', 1, 0), ('PVN', 1, 0), ('PVA', 0, 1), ('PVT', 1, 0), ('SM', 1, 1), ('PVN', 0, 1),
    ('PVT', 0, 1), ('PVN', 1, 1), ('PVT', 1, 1), ('PVA', 1, 1), ('FIN', 0), ('OP', 0), ('FIN', 1),
    ('OP', 1),
)
_ORDER_FIRST = (
    ('QP', 0), ('DX',), ('QP', 1), ('DK',), ('QK', 0, 0), ('DV',), ('QK', 0, 1), ('SM', 0, 0), ('DW',),
    ('QK', 1, 0), ('SM', 0, 1), ('QK', 1, 1), ('SM', 1, 0), ('PVA', 0, 0), ('PVN', 0, 0), ('PVT', 0, 0),
    ('SM', 1, 1), ('PVA', 0, 1), ('PVN', 0, 1), ('PVT', 0, 1), ('PVA', 1, 0), ('PVN', 1, 0), ('PVT', 1, 0),
    ('FIN', 0), ('PVA', 1, 1), ('PVN', 1, 1), ('PVT', 1, 1), ('OP', 0), ('FIN', 1), ('OP', 1),
)


def _mm(a, b, dn=NN):
    return jax.lax.dot_general(a, b, dn, preferred_element_type=F32)


def _kernel(xa, ka, va, wqa, woa, xb, kb, vb, wqb, wob, out_hbm,
            xbuf, kvbuf, wqbuf, wobuf, acc_ref, obuf, sem, *, Dh, NP, B, Sq, D):
    hps = HPS
    XH = (xa, xb); KVH = ((ka, kb), (va, vb)); WQH = (wqa, wqb); WOH = (woa, wob)
    PW = 2 * Dh
    NG = NP // hps
    NS = 2 * hps
    LB = B.bit_length() - 1
    scale = float(Dh ** -0.5 * LOG2E)

    xsem = lambda i: sem.at[i]
    ksem = lambda i: sem.at[NS + i]
    vsem = lambda i: sem.at[2 * NS + i]
    wqsem = lambda i: sem.at[3 * NS + i]
    wosem = lambda i: sem.at[4 * NS + 1 + i]
    osem = lambda i: sem.at[5 * NS + 2 + i]

    def rcopy(src, dst, s, nlead):
        lead = (slice(None),) * nlead
        for half in range(2):
            pltpu.make_async_copy(src.at[lead + (slice(None), half)],
                                  dst.at[lead + (slice(None), slice(None), pl.ds(half * 8, 8))], s).start()

    def ld2d(tile_col, R2, J):
        cols = [pltpu.bitcast(tile_col(c).reshape(R2 * 8, 128), BF16) for c in range(J)]
        return jnp.concatenate(cols, axis=1)

    x32 = xbuf.bitcast(jnp.uint32); kv32 = kvbuf.bitcast(jnp.uint32)
    wq32 = wqbuf.bitcast(jnp.uint32); wo32 = wobuf.bitcast(jnp.uint32)

    def x_start(b, cs):
        for r in range(2):
            rcopy(XH[r].at[b], xbuf.at[cs, r], xsem(cs), 0)

    def kv_start(kv, p, npair, b, ks, j0, si=None):
        si = ks * hps + j0 if si is None else si
        for r in range(2):
            rcopy(KVH[kv][r].at[b, pl.ds(p, npair)], kvbuf.at[ks, kv, r, pl.ds(j0, npair)], (ksem, vsem)[kv](si), 2)

    def x_wait(cs):
        pltpu.make_async_copy(xbuf.at[cs], xbuf.at[cs], xsem(cs)).wait()

    def kv_wait(ks, j0, npair, which=(0, 1)):
        for kv in which:
            v = kvbuf.at[ks, kv, :, pl.ds(j0, npair)]
            pltpu.make_async_copy(v, v, (ksem, vsem)[kv](ks * hps + j0)).wait()

    def w_rows_start(p, npair, ws, j0, q0, nq, o0, no, which='qo'):
        if 'q' in which:
            for r in range(2):
                rcopy(WQH[r].at[pl.ds(q0 // 16, nq // 16), :, pl.ds(p * 3, 3 * npair)],
                      wqbuf.at[ws, r, pl.ds(q0 // 16, nq // 16), pl.ds(j0 * 3, 3 * npair)], wqsem(ws * hps + j0), 0)
        if 'o' in which:
            for r in range(2):
                rcopy(WOH[r].at[pl.ds(p * (PW // 16) + o0 // 16, no // 16)],
                      wobuf.at[ws, r, pl.ds(j0 * (PW // 16) + o0 // 16, no // 16)], wosem(ws * hps + j0), 0)

    def w_slice_start(p, npair, b, ws, j0):
        rq = D // B; ro = npair * PW // B
        w_rows_start(p, npair, ws, j0, pl.multiple_of(b * rq, 16), rq, pl.multiple_of(b * ro, 16), ro)

    def w_wait(ws, j0, npair, which='qo'):
        if 'q' in which:
            for r in range(2):
                v = wqbuf.at[ws, r, :, pl.ds(j0 * 3, 3 * npair)]
                pltpu.make_async_copy(v, v, wqsem(ws * hps + j0)).wait()
        if 'o' in which:
            for r in range(2):
                v = wobuf.at[ws, r, pl.ds(j0 * (PW // 16), npair * PW // 16)]
                pltpu.make_async_copy(v, v, wosem(ws * hps + j0)).wait()

    def o_wait(slot):
        pltpu.make_async_copy(obuf.at[slot], obuf.at[slot], osem(slot)).wait()

    def compute(first, b, xs, ks, j0, ws, jw0, npair, seq, hooks):
        st = {}

        def QP(u):
            r, j = u % 2, u // 2
            x = ld2d(lambda c: x32[xs, r, :, c], Sq // 16, D // 128)
            w = ld2d(lambda c: wq32[ws, r, :, (jw0 + j) * 3 + c], D // 16, 3)
            st['q', u] = (_mm(x, w) * scale).astype(BF16)

        def kv_rows(kv, r, j, h, r0, nr):
            return ld2d(lambda c: kv32[ks, kv, r, j0 + j, h, pl.ds(r0, nr), c], nr, kvbuf.shape[-3])

        def QK(u, h):
            r, j = u % 2, u // 2
            kt = kv_rows(0, r, j, h, 0, Dh // 16)
            z = jnp.zeros((256 - Dh, kt.shape[1]), BF16)
            kt = jnp.concatenate([kt, z] if h == 0 else [z, kt], axis=0)
            st['s', u, h] = _mm(st['q', u][:, h * 128:h * 128 + 256], kt)

        def SM(u, h):
            s = st['s', u, h]
            m = jnp.max(s, axis=-1, keepdims=True)
            e = jnp.exp2(s - m)
            st['l', u, h] = jnp.sum(e, axis=-1, keepdims=True)
            st['p', u, h] = e.astype(BF16)

        def PVA(u, h):
            r, j = u % 2, u // 2
            st['oa', u, h] = _mm(kv_rows(1, r, j, h, 0, Dh // 16), st['p', u, h][:QS], NT)

        def PVN(u, h):
            r, j = u % 2, u // 2
            st['on', u, h] = _mm(st['p', u, h][QS:], kv_rows(1, r, j, h, 0, 8), NT)

        def PVT(u, h):
            r, j = u % 2, u // 2
            st['ot', u, h] = _mm(kv_rows(1, r, j, h, 8, Dh // 16 - 8), st['p', u, h][QS:], NT)

        def FIN(u):
            il0 = 1.0 / st['l', u, 0]; il1 = 1.0 / st['l', u, 1]
            lane = jax.lax.broadcasted_iota(jnp.int32, (Sq, 128), 1)
            ilm = jnp.where(lane < Dh - 128, il0, il1)
            a0, a1 = st['oa', u, 0], st['oa', u, 1]
            am = jnp.concatenate([a0[128:], a1[128:]], axis=0)
            bm = jnp.concatenate([st['ot', u, 0], st['ot', u, 1]], axis=0)
            t0 = jnp.concatenate([a0[:128].T, st['on', u, 0]], axis=0) * il0
            t1 = jnp.concatenate([am.T, bm.T], axis=0) * ilm
            t2 = jnp.concatenate([a1[:128].T, st['on', u, 1]], axis=0) * il1
            st['o', u] = jnp.concatenate([t0.astype(BF16), t1.astype(BF16), t2.astype(BF16)], axis=1)

        def OP(u):
            r, j = u % 2, u // 2
            base = (jw0 + j) * (PW // 16)
            rows = ((0, 12), (20, 4), (12, 8))
            w = ld2d(lambda c: jnp.concatenate([wo32[ws, r, pl.ds(base + a, n), c] for a, n in rows], axis=0),
                     PW // 16, D // 128)
            y = _mm(st['o', u], w)
            if j < npair - 1:
                st['y', r] = y if j == 0 else st['y', r] + y
            else:
                if j > 0:
                    y = st['y', r] + y
                if first is not True:
                    old = acc_ref[b, :, r * D:(r + 1) * D]
                    if first is not False:
                        old = jnp.where(first, 0.0, old)
                    y = y + old
                acc_ref[b, :, r * D:(r + 1) * D] = y

        ops = dict(QP=QP, QK=QK, SM=SM, PVA=PVA, PVN=PVN, PVT=PVT, FIN=FIN, OP=OP, **hooks)
        for f, *a in seq:
            ops[f](*a)

    npre = min(NS, NFG + hps)
    x_start(0, 0)
    w_rows_start(0, 1, 0, 0, 0, D, 0, PW, 'q')
    kv_start(0, 0, 1, 0, 0, 0)
    kv_start(1, 0, 1, 0, 0, 0)
    w_rows_start(0, 1, 0, 0, 0, D, 0, PW, 'o')
    for k in range(1, npre):
        x_start(k, k)
        kv_start(0, 0, 1, k, k // hps, k % hps)
        kv_start(1, 0, 1, k, k // hps, k % hps)

    for c0 in range(NFG):
        seq = []; seen = set()
        for op in _ORDER_FIRST:
            if op[0][0] == 'D':
                if c0 + hps >= npre and op[0] != 'DW':
                    seq.append(op)
                continue
            kind = 'PV' if op[0].startswith('PV') else op[0]
            if kind not in seen:
                seen.add(kind)
                if kind == 'QP': seq.append(('WX',))
                if kind == 'QK' and c0 == 0: seq.append(('WK',))
                if kind == 'PV': seq.append(('WV',))
                if kind == 'OP' and c0 == 0: seq.append(('WO',))
            seq.append(op)
        n_ = c0 + hps; ncs = n_ % NS

        def wx(c0=c0):
            x_wait(c0)
            if c0 == 0:
                w_wait(0, 0, 1, 'q')
            else:
                kv_wait(c0 // hps, c0 % hps, 1, (0,))

        hooks = dict(DX=lambda: x_start(n_, ncs),
                     DK=lambda: kv_start(0, 0, 1, n_, ncs // hps, ncs % hps),
                     DV=lambda: kv_start(1, 0, 1, n_, ncs // hps, ncs % hps),
                     WX=wx, WK=lambda: kv_wait(c0 // hps, c0 % hps, 1, (0,)),
                     WV=lambda: kv_wait(c0 // hps, c0 % hps, 1, (1,)), WO=lambda: w_wait(0, 0, 1, 'o'))
        compute(True, c0, c0, c0 // hps, c0 % hps, 0, 0, 1, seq, hooks)
    for c0 in range(NFG):
        for pp in (1, 2):
            w_slice_start(pp, 1, c0, pp // hps, pp % hps)

    def ramp_pair(p, c):
        @pl.when(p > 0)
        def _():
            w_wait(0, p, 1)

        def step(b, c):
            cidx = p * B + b
            cs = jax.lax.rem(cidx, NS)
            wrap = (b + hps >= B)
            np_ = jnp.where(wrap, p + 1, p); nb = jnp.where(wrap, b + hps - B, b + hps)
            is_tr = jnp.logical_and(wrap, p == hps - 1)
            np_ = jnp.where(is_tr, hps + (b + hps - B), np_); nb = jnp.where(is_tr, 0, nb)
            ncs = jax.lax.rem(cidx + hps, NS)
            nks = ncs // hps; nj = jax.lax.rem(ncs, hps)
            nsem = jnp.where(is_tr, 0, ncs)
            pa = 2 * p + 1

            def DW():
                for pp in (pa, pa + 1):
                    w_slice_start(pp, 1, b, pp // hps, jax.lax.rem(pp, hps))

            hooks = dict(DX=lambda: x_start(nb, ncs), DK=lambda: kv_start(0, np_, 1, nb, nks, nj, nsem),
                         DV=lambda: kv_start(1, np_, 1, nb, nks, nj, nsem), DW=DW)
            ks = cs // hps; j = jax.lax.rem(cs, hps)
            x_wait(cs)
            kv_wait(ks, j, 1)
            compute(p == 0, b, cs, ks, j, 0, p, 1, _ORDER_RAMP, hooks)
            return c

        jax.lax.fori_loop(jnp.where(p == 0, NFG, 0), B, step, 0)
        return c

    jax.lax.fori_loop(0, hps, ramp_pair, 0)

    def finalize(g, b):
        @pl.when(g == NG - 1)
        def _():
            so = jnp.bitwise_and(b, 1)

            @pl.when(b >= 2)
            def _():
                o_wait(so)

            RC = 48

            def cvt(i, c):
                rows = pl.ds(pl.multiple_of(i * RC, RC), RC)
                obuf[so, rows, :] = acc_ref[b, rows, :].astype(BF16)
                pltpu.make_async_copy(obuf.at[so, rows], out_hbm.at[b, rows], osem(so)).start()
                return c

            jax.lax.fori_loop(0, Sq // RC, cvt, 0)

    def main_group(g, c):
        gs = jnp.bitwise_and(g, 1)
        g1 = jnp.minimum(g + 1, NG - 1)

        @pl.when(g == 1)
        def _():
            for j in range(hps):
                w_wait(1, j, 1)

        @pl.when(g > 1)
        def _():
            w_wait(gs, 0, hps)

        def step(b, c):
            ks = jnp.bitwise_and(b, 1)
            nb = jnp.bitwise_and(b + 1, B - 1)
            ng = jnp.minimum(g + jax.lax.shift_right_logical(b + 1, LB), NG - 1)
            hooks = dict(DX=lambda: x_start(nb, (1 - ks) * hps),
                         DK=lambda: kv_start(0, ng * hps, hps, nb, 1 - ks, 0),
                         DV=lambda: kv_start(1, ng * hps, hps, nb, 1 - ks, 0),
                         DW=lambda: w_slice_start(g1 * hps, hps, b, 1 - gs, 0))
            x_wait(ks * hps)
            kv_wait(ks, 0, hps)
            compute(False, b, ks * hps, ks, 0, gs, 0, hps, _ORDER_MAIN, hooks)
            finalize(g, b)
            return c

        jax.lax.fori_loop(0, B, step, 0)
        return c

    for k in range(1, hps):
        x_wait(k)
    jax.lax.fori_loop(1, NG, main_group, 0)
    w_wait(2, 0, 1)
    x_wait(0)
    kv_wait(0, 0, hps)
    w_wait(NG % 2, 0, hps)
    o_wait(0)
    o_wait(1)


def _tiles(a):
    *lead, R, C = a.shape
    n = len(lead)
    a = a.reshape(*lead, R // 16, 2, 8, C // 128, 128)
    return a.transpose(*range(n), n, n + 1, n + 3, n + 2, n + 4)


@jax.jit
def pallas_concat_heads__gqa_block_cached__gqa_block_cached__near_ridge_kernel(
        A_x, A_k_cache, A_v_cache, A_wq, A_wo, B_x, B_k_cache, B_v_cache, B_wq, B_wo):
    B, Sq, D = A_x.shape
    _, H, Sk, Dh = A_k_cache.shape
    NP = H // 2
    NS = 2 * HPS
    assert Dh == 192 and H % (2 * HPS) == 0 and NP // HPS >= 3 and B >= 4 and B & (B - 1) == 0
    assert Sq % 48 == 0 and Sq > QS and D % (16 * B) == 0 and D % 128 == 0 and Sk % 128 == 0

    def kt(a):
        return _tiles(jnp.swapaxes(a, 2, 3).reshape(B, NP, 2, Dh, Sk))

    def vshape(lead, R, C):
        return lead + (R // 16, C // 128, 16, 128)

    anys = pl.BlockSpec(memory_space=pl.ANY)
    return pl.pallas_call(
        functools.partial(_kernel, Dh=Dh, NP=NP, B=B, Sq=Sq, D=D),
        in_specs=[anys] * 10,
        out_specs=anys,
        out_shape=jax.ShapeDtypeStruct((B, Sq, 2 * D), A_x.dtype),
        scratch_shapes=[
            pltpu.VMEM(vshape((NS, 2), Sq, D), BF16),
            pltpu.VMEM(vshape((2, 2, 2, HPS, 2), Dh, Sk), BF16),
            pltpu.VMEM(vshape((3, 2), D, HPS * 2 * Dh), BF16),
            pltpu.VMEM(vshape((3, 2), HPS * 2 * Dh, D), BF16),
            pltpu.VMEM((B, Sq, 2 * D), F32),
            pltpu.VMEM((2, Sq, 2 * D), BF16),
            pltpu.SemaphoreType.DMA((5 * NS + 4,)),
        ],
        compiler_params=pltpu.CompilerParams(vmem_limit_bytes=110 * 1024 * 1024, disable_bounds_checks=True),
    )(_tiles(A_x), kt(A_k_cache), kt(A_v_cache), _tiles(A_wq), _tiles(A_wo),
      _tiles(B_x), kt(B_k_cache), kt(B_v_cache), _tiles(B_wq), _tiles(B_wo))
```
